```python
import jax
import jax.numpy as jnp

def _softmax(x, axis=-1):
    return jax.nn.softmax(x, axis=axis)
def _gelu(x):
    return jax.nn.gelu(x, approximate=True)
def _silu(x):
    return jax.nn.silu(x)
def _sigmoid(x):
    return jax.nn.sigmoid(x)
def _layernorm(x, axis=-1, eps=1e-5):
    m = jnp.mean(x, axis=axis, keepdims=True)
    v = jnp.var(x, axis=axis, keepdims=True)
    return (x - m) / jnp.sqrt(v + eps)
def _scatter_add(tgt, idx, src, axis=0):
    return tgt.at[idx].add(src)
def _segment_sum(src, seg, n):
    return jax.ops.segment_sum(src, seg, n)
class _Rng:
    def __init__(self, key):
        self._k = key
    def _next(self):
        self._k, sub = jax.random.split(self._k)
        return sub
    def normal(self, shape):
        return jax.random.normal(self._next(), shape, dtype=jnp.bfloat16)
    def randint(self, lo, hi, shape):
        return jax.random.randint(self._next(), shape, lo, hi, dtype=jnp.int32)
    def uniform(self, shape, lo=0.0, hi=1.0):
        return jax.random.uniform(self._next(), shape, jnp.bfloat16, lo, hi)
    def permutation(self, n):
        return jax.random.permutation(self._next(), n)


kernel_name = 'interleave_layers__softmax_full_mha__ssm_conv_h3__prompt'

def setup_inputs():
    _rng = _Rng(jax.random.key(int.from_bytes(__import__("os").urandom(4), "little")))
    _w = (lambda a: (lambda t: t.astype(jnp.bfloat16) if jnp.issubdtype(t.dtype, jnp.floating) else t)(jnp.asarray(a)))
    def _A_setup():
        B, S, D = 1, 2048, 1024
        return {
            "x": _w((lambda *s: _rng.normal(s) * 0.05)(B, S, D)),
            "wqkv": _w((lambda *s: _rng.normal(s) * 0.05)(D, 3 * D)),
            "wo": _w((lambda *s: _rng.normal(s) * 0.05)(D, D)),
        }
    _A_in = _A_setup()

    def _B_setup():
        B, S, D = 1, 2048, 1024
        ks = 4
        return {
            "q": _w((lambda *s: _rng.normal(s) * 0.05)(B, S, D)),
            "k": _w((lambda *s: _rng.normal(s) * 0.05)(B, S, D)),
            "v": _w((lambda *s: _rng.normal(s) * 0.05)(B, S, D)),
            "shift_k": _w((lambda *s: _rng.normal(s) * 0.05)(D, ks) * 0.5),
            "ssm_k": _w((lambda *s: _rng.normal(s) * 0.05)(D, S) * (1.0 / S ** 0.5)),
            "ssm_D": _w((lambda *s: _rng.normal(s) * 0.05)(D)),
        }
    _B_in = _B_setup()

    return {
        "A_x": _A_in["x"],
        "A_wqkv": _A_in["wqkv"],
        "A_wo": _A_in["wo"],
        "B_q": _B_in["q"],
        "B_k": _B_in["k"],
        "B_v": _B_in["v"],
        "B_shift_k": _B_in["shift_k"],
        "B_ssm_k": _B_in["ssm_k"],
        "B_ssm_D": _B_in["ssm_D"],
    }

def reference(A_x, A_wqkv, A_wo, B_q, B_k, B_v, B_shift_k, B_ssm_k, B_ssm_D):
    def _A_ref(x, wqkv, wo):
        B, S, D = x.shape
        H = 32; Dh = D // H
        qkv = (lambda x, *d: x.transpose(*d))((x @ wqkv).reshape(B, S, 3, H, Dh), 2, 0, 3, 1, 4)
        q, k, v = qkv[0], qkv[1], qkv[2]
        scale = Dh ** -0.5
        scores = jnp.einsum("bhqd,bhkd->bhqk", q, k) * scale
        p = _softmax(scores, axis=-1)
        o = jnp.einsum("bhqk,bhkd->bhqd", p, v)
        return (lambda x, *d: x.transpose(*d))(o, 0, 2, 1, 3).reshape(B, S, D) @ wo

    def _B_ref(q, k, v, shift_k, ssm_k, ssm_D):
        B, S, D = q.shape
        ks = shift_k.shape[-1]
        k_pad = jnp.pad(k, ((0, 0), (ks - 1, 0), (0, 0)))
        k_shift = jnp.zeros_like(k)
        for t in range(ks):
            k_shift = k_shift + k_pad[:, t:t + S, :] * shift_k[:, ks - 1 - t][None, None, :]
        kv = k_shift * v
        L = 2 * S
        kv_pad = jnp.pad(kv, ((0, 0), (0, S), (0, 0)))
        kf_pad = jnp.pad(ssm_k, ((0, 0), (0, S)))
        kv_f = (lambda x, axes=(-2,-1): jnp.fft.rfft2(x.astype(jnp.float32), axes=axes))(kv_pad[:, None, :, :], axes=(1, 2))
        kf_f = (lambda x, axes=(-2,-1): jnp.fft.rfft2(x.astype(jnp.float32), axes=axes))(kf_pad[:, None, :], axes=(1, 2))
        kf_f = (lambda x, *d: x.transpose(*d))(kf_f, 1, 2, 0)
        y_f = kv_f * kf_f[None, :, :, :]
        y = (lambda x, s, axes=(-2,-1): jnp.fft.irfft2(x, s=s, axes=axes).astype(jnp.bfloat16))(y_f, (1, L), axes=(1, 2))[:, 0, :S, :]
        y = y + kv * ssm_D[None, None, :]
        return q * y

    x = A_x
    x = x + _A_ref(_layernorm(x, axis=-1), A_wqkv, A_wo)
    x = x + _B_ref(_layernorm(x, axis=-1), B_k, B_v, B_shift_k, B_ssm_k, B_ssm_D)
    x = x + _A_ref(_layernorm(x, axis=-1), A_wqkv, A_wo)
    x = x + _B_ref(_layernorm(x, axis=-1), B_k, B_v, B_shift_k, B_ssm_k, B_ssm_D)
    return x
```

```python
import functools
import numpy as np
import jax
import jax.numpy as jnp
import jax.experimental.pallas as pl
import jax.experimental.pallas.tpu as pltpu

S, D, H, DH, KS = 2048, 1024, 32, 32, 4
BQ, CK, RB, CT = 512, 128, 512, 256
R = 72
F32, BF16, U32 = jnp.float32, jnp.bfloat16, jnp.uint32


def _dft_consts():
    n = 4096
    k1 = np.arange(33)[:, None]
    n1 = np.arange(32)[None, :]
    f1 = np.zeros((R, 32))
    f1[0:66:2] = np.cos(2 * np.pi * k1 * n1 / 64)
    f1[1:66:2] = -np.sin(2 * np.pi * k1 * n1 / 64)
    wgt = np.where((k1 == 0) | (k1 == 32), 1.0, 2.0)
    fi = np.zeros((32, R))
    fi[:, 0:66:2] = (wgt * np.cos(2 * np.pi * k1 * n1 / 64)).T / 64
    fi[:, 1:66:2] = (-wgt * np.sin(2 * np.pi * k1 * n1 / 64)).T / 64
    a = np.arange(64)
    g = np.zeros((33, 128, 128))
    gi = np.zeros((33, 128, 128))
    for k in range(33):
        w = np.exp(-2j * np.pi * (a[:, None] * a[None, :] / 64 + k * a[None, :] / n))
        g[k] = np.block([[w.real, -w.imag], [w.imag, w.real]])
        wi = np.conj(w).T / 64
        gi[k] = np.block([[wi.real, -wi.imag], [wi.imag, wi.real]])
    return [x.astype(np.float32) for x in (f1, fi, g, gi)]


def _pk(x):
    return pltpu.bitcast(x, U32)


def _upk(x):
    return pltpu.bitcast(x, BF16)


def _dot(a, b):
    return jnp.dot(a, b, preferred_element_type=F32)


def _ln(x):
    m = jnp.mean(x, axis=-1, keepdims=True)
    d = x - m
    v = jnp.mean(d * d, axis=-1, keepdims=True)
    return d * jax.lax.rsqrt(v + 1e-5)


def _ds(i, n):
    return pl.ds(pl.multiple_of(i * n, n), n)


def _ld(ref, rows, js):
    return jnp.concatenate([ref[j, rows, :] for j in js], axis=1)


def _st(ref, rows, js, val):
    for i, j in enumerate(js):
        ref[j, rows, :] = val[:, i * 128:(i + 1) * 128]


def _conv(k_ref, v_ref, sk_ref, h_ref, sd_ref, f1_ref, fi_ref, g_ref, gi_ref, y_ref,
          xin, abuf, bbuf, kpad):
    bbuf[:, 66 * 64:, :] = jnp.zeros((2, (R - 66) * 64, 128), F32)
    kpad[0:8, :] = jnp.zeros((8, CT), F32)

    def tile(c, carry):
        cs = _ds(c, CT)
        kpad[8:, :] = k_ref[:, cs].astype(F32)

        def prep(r, carry):
            rows = _ds(r, 128)
            hb = h_ref[cs, rows].astype(F32)
            _st(xin, rows, (2, 3), hb.T)
            return carry
        jax.lax.fori_loop(0, S // 128, prep, 0)
        sk = sk_ref[:, cs]
        for r in range(S // 256):
            acc = None
            for t in range(KS):
                o = 8 - (KS - 1) + t + r * 256
                term = kpad[o:o + 256, :] * sk[KS - 1 - t:KS - t, :]
                acc = term if acc is None else acc + term
            _st(xin, slice(r * 256, (r + 1) * 256), (0, 1), acc * v_ref[r * 256:(r + 1) * 256, cs].astype(F32))

        def s1(i, carry):
            for u in range(8):
                n2 = i * 8 + u
                x = _ld(xin, pl.ds(n2, 32, stride=64), range(4)).astype(BF16)
                _st(abuf, pl.ds(n2, R, stride=64), range(4), _dot(f1_ref[...], x))
            return carry
        jax.lax.fori_loop(0, 8, s1, 0)

        def s2(i, carry):
            for u in range(3):
                k1 = i * 3 + u
                rows = _ds(k1, 128)
                z = _dot(g_ref[k1], _ld(abuf, rows, range(4)).astype(BF16))
                xr, xi = z[:64, :CT], z[64:, :CT]
                hr, hi = z[:64, CT:], z[64:, CT:]
                yy = jnp.concatenate([xr * hr - xi * hi, xr * hi + xi * hr], axis=0)
                _st(bbuf, rows, (0, 1), _dot(gi_ref[k1], yy.astype(BF16)))
            return carry
        jax.lax.fori_loop(0, 11, s2, 0)

        def s3(i, carry):
            for u in range(8):
                n2 = i * 8 + u
                b = _ld(bbuf, pl.ds(n2, R, stride=64), (0, 1)).astype(BF16)
                _st(xin, pl.ds(n2, 32, stride=64), (2, 3), _dot(fi_ref[...], b))
            return carry
        jax.lax.fori_loop(0, 8, s3, 0)
        sd = sd_ref[:, cs]
        for r in range(S // 256):
            rows = slice(r * 256, (r + 1) * 256)
            y_ref[rows, cs] = (_ld(xin, rows, (2, 3)) + _ld(xin, rows, (0, 1)) * sd).astype(BF16)
        return carry
    jax.lax.fori_loop(0, D // CT, tile, 0)


def _attention(qt_ref, k_ref, vt_ref, ot_ref, sb, pb, kb, qb, ml):
    nq = S // BQ
    nst = H * nq

    def stage(t):
        t = jnp.minimum(t, nst - 1)
        h = t // nq
        j = t % nq
        q = qt_ref[_ds(h // 4, 64), _ds(j, BQ)]
        r = jax.lax.broadcasted_iota(jnp.int32, (64, BQ), 0)
        qb[...] = jnp.where((r >> 4) == h % 4, q, jnp.uint32(0))

        @pl.when(t % (4 * nq) == 0)
        def _():
            kb[...] = k_ref[h // 4]

    def step(t, sn, sc, pc, pp):
        tp = jnp.maximum(t - 1, 0)
        hp = tp // nq
        jp = tp % nq
        vt = vt_ref[_ds(hp, 16), :]
        qm = _upk(qb[...])
        m = ml[0:1]
        m8 = l8 = acc = dep = None
        for c in range(S // CK):
            rows = slice(c * CK, (c + 1) * CK)
            prows = slice(c * CK // 2, (c + 1) * CK // 2)
            kc = kb[prows, :]
            if dep is not None:
                kc = jnp.where(jnp.tile(dep, (CK // 16, 1)), jnp.uint32(0), kc)
            s = _dot(_upk(kc), qm)
            sn[rows, :] = s
            mc = jnp.max(s.reshape(CK // 8, 8, BQ), axis=0)
            m8 = mc if m8 is None else jnp.maximum(m8, mc)
            a = _dot(_upk(vt[:, rows]), _upk(pp[prows, :]))
            acc = a if acc is None else acc + a
            p = jnp.exp2(sc[rows, :] - m)
            pc[prows, :] = _pk(p.astype(BF16))
            lc = jnp.sum(p.reshape(CK // 8, 8, BQ), axis=0)
            l8 = lc if l8 is None else l8 + lc
            dep = functools.reduce(
                jnp.minimum, [lc[:, i * 128:(i + 1) * 128] for i in range(BQ // 128)]) < -1.0
        ot_ref[_ds(hp, 32), _ds(jp, BQ)] = (acc / ml[1:2]).astype(BF16)
        ml[0:1] = jnp.max(m8, axis=0, keepdims=True)
        ml[1:2] = jnp.sum(l8, axis=0, keepdims=True)

    stage(0)
    qm = _upk(qb[...])
    m8 = None
    for c in range(S // 512):
        s = _dot(_upk(kb[c * 256:(c + 1) * 256, :]), qm)
        sb[0][c * 512:(c + 1) * 512, :] = s
        mc = jnp.max(s.reshape(64, 8, BQ), axis=0)
        m8 = mc if m8 is None else jnp.maximum(m8, mc)
    ml[0:1] = jnp.max(m8, axis=0, keepdims=True)
    ml[1:2] = jnp.ones((1, BQ), F32)
    pb[1][...] = jnp.zeros(pb[1].shape, U32)
    stage(1)

    def body(t, carry):
        for par in (0, 1):
            @pl.when(t % 2 == par)
            def _():
                step(t, sb[1 - par], sb[par], pb[par], pb[1 - par])
        stage(t + 2)
        return carry
    jax.lax.fori_loop(0, nst, body, 0)
    a = _dot(_upk(vt_ref[(H - 1) * 16:H * 16, :]), _upk(pb[1][...]))
    ot_ref[(H - 1) * 32:, (nq - 1) * BQ:] = (a / ml[1:2]).astype(BF16)


def _kernel(x_ref, wqkv_ref, wo_ref, k_ref, v_ref, sk_ref, h_ref, sd_ref,
            f1_ref, fi_ref, g_ref, gi_ref, o_ref,
            xr, y, wt, qt, kk, vt, ot, s0, s1, p0, p1, kb, qb, ml, xin, abuf, bbuf, kpad):
    _conv(k_ref, v_ref, sk_ref, h_ref, sd_ref, f1_ref, fi_ref, g_ref, gi_ref, y,
          xin, abuf, bbuf, kpad)

    def wtr(i, carry):
        for s, o in ((0, 0), (2 * D, D)):
            w = wqkv_ref[:, pl.ds(pl.multiple_of(s + i * 128, 128), 128)].astype(F32)
            wt[pl.ds(pl.multiple_of(o + i * 128, 128), 128), :] = w.T.astype(BF16)
        return carry
    jax.lax.fori_loop(0, D // 128, wtr, 0)
    xr[...] = x_ref[...].astype(F32)
    qscale = float(DH ** -0.5 * np.log2(np.e))
    nt = (((1,), (1,)), ((), ()))

    def layer(li, carry):
        def proj(r, carry):
            rows = _ds(r, RB)
            h = _ln(xr[rows, :]).astype(BF16)
            qv = jax.lax.dot_general(wt[...], h, nt, preferred_element_type=F32)
            qt[:, rows] = _pk((qv[:D] * qscale).astype(BF16))
            vt[:, rows] = _pk(qv[D:].astype(BF16))
            kx = _pk(_dot(h, wqkv_ref[:, D:2 * D]).astype(BF16))
            for g in range(8):
                kk[g, _ds(r, RB // 2), :] = kx[:, g * 128:(g + 1) * 128]
            return carry
        jax.lax.fori_loop(0, S // RB, proj, 0)
        _attention(qt, kk, vt, ot, (s0, s1), (p0, p1), kb, qb, ml)

        def post(r, carry):
            rows = _ds(r, RB)
            a = jax.lax.dot_general(ot[:, rows], wo_ref[...], (((0,), (0,)), ((), ())),
                                    preferred_element_type=F32)
            x = xr[rows, :] + a
            x = x + _ln(x) * y[rows, :].astype(F32)
            xr[rows, :] = x
            o_ref[rows, :] = x.astype(BF16)
            return carry
        jax.lax.fori_loop(0, S // RB, post, 0)
        return carry
    jax.lax.fori_loop(0, 2, layer, 0)


@jax.jit
def pallas_interleave_layers__softmax_full_mha__ssm_conv_h3__prompt_kernel(
    A_x, A_wqkv, A_wo, B_q, B_k, B_v, B_shift_k, B_ssm_k, B_ssm_D,
):
    V = pltpu.VMEM
    consts = [c.astype(BF16) for c in _dft_consts()]
    out = pl.pallas_call(
        _kernel,
        out_shape=jax.ShapeDtypeStruct((S, D), BF16),
        scratch_shapes=[
            V((S, D), F32), V((S, D), BF16), V((2 * D, D), BF16),
            V((D // 2, S), U32), V((8, S // 2, 128), U32), V((D // 2, S), U32), V((D, S), BF16),
            V((S, BQ), F32), V((S, BQ), F32), V((S // 2, BQ), U32), V((S // 2, BQ), U32),
            V((S // 2, 128), U32), V((64, BQ), U32), V((8, BQ), F32),
            V((4, S, 128), F32), V((4, R * 64, 128), F32), V((2, R * 64, 128), F32),
            V((S + 8, CT), F32),
        ],
        compiler_params=pltpu.CompilerParams(vmem_limit_bytes=120 << 20),
    )(A_x.reshape(S, D), A_wqkv, A_wo, B_k.reshape(S, D), B_v.reshape(S, D),
      B_shift_k.T.astype(F32), B_ssm_k, B_ssm_D.reshape(1, D).astype(F32), *consts)
    return out.reshape(1, S, D)
```

```python
import functools
import numpy as np
import jax
import jax.numpy as jnp
import jax.experimental.pallas as pl
import jax.experimental.pallas.tpu as pltpu

S, D, H, DH, KS = 2048, 1024, 32, 32, 4
BQ, CK, RB, CT = 512, 128, 512, 256
R = 72
P = 65
F32, BF16, U32 = jnp.float32, jnp.bfloat16, jnp.uint32


def _dft_consts():
    n = 4096
    k1 = np.arange(33)[:, None]
    n1 = np.arange(32)[None, :]
    f1 = np.zeros((R, 32))
    f1[0:66:2] = np.cos(2 * np.pi * k1 * n1 / 64)
    f1[1:66:2] = -np.sin(2 * np.pi * k1 * n1 / 64)
    wgt = np.where((k1 == 0) | (k1 == 32), 1.0, 2.0)
    fi = np.zeros((32, R))
    fi[:, 0:66:2] = (wgt * np.cos(2 * np.pi * k1 * n1 / 64)).T / 64
    fi[:, 1:66:2] = (-wgt * np.sin(2 * np.pi * k1 * n1 / 64)).T / 64
    a = np.arange(64)
    g = np.zeros((33, 128, 128))
    gi = np.zeros((33, 128, 128))
    for k in range(33):
        w = np.exp(-2j * np.pi * (a[:, None] * a[None, :] / 64 + k * a[None, :] / n))
        g[k] = np.block([[w.real, -w.imag], [w.imag, w.real]])
        wi = np.conj(w).T / 64
        gi[k] = np.block([[wi.real, -wi.imag], [wi.imag, wi.real]])
    return [x.astype(np.float32) for x in (f1, fi, g, gi)]


def _pk(x):
    return pltpu.bitcast(x, U32)


def _upk(x):
    return pltpu.bitcast(x, BF16)


def _dot(a, b):
    return jnp.dot(a, b, preferred_element_type=F32)


def _ln(x):
    m = jnp.mean(x, axis=-1, keepdims=True)
    d = x - m
    v = jnp.mean(d * d, axis=-1, keepdims=True)
    return d * jax.lax.rsqrt(v + 1e-5)


def _ds(i, n):
    return pl.ds(pl.multiple_of(i * n, n), n)


def _ld(ref, rows, js):
    return jnp.concatenate([ref[j, rows, :] for j in js], axis=1)


def _st(ref, rows, js, val):
    for i, j in enumerate(js):
        ref[j, rows, :] = val[:, i * 128:(i + 1) * 128]


def _conv(k_ref, v_ref, sk_ref, h_ref, sd_ref, f1_ref, fi_ref, g_ref, gi_ref, y_ref,
          xin, abuf, bbuf, kpad, wait_tile):
    bbuf[:, 66 * P:, :] = jnp.zeros((2, (R - 66) * P, 128), F32)
    kpad[0:8, :] = jnp.zeros((8, CT), F32)

    def tile(c, carry):
        cs = _ds(c, CT)
        wait_tile(c)
        kpad[8:, :] = k_ref[:, cs].astype(F32)

        def prep(r, carry):
            rows = _ds(r, 128)
            hb = h_ref[cs, rows].astype(F32)
            ht = hb.T
            for u in range(2):
                _st(xin, pl.ds((2 * r + u) * P, 64), (2, 3), ht[u * 64:(u + 1) * 64])
            return carry
        jax.lax.fori_loop(0, S // 128, prep, 0)
        sk = sk_ref[:, cs]
        for r in range(S // 64):
            acc = None
            for t in range(KS):
                o = 8 - (KS - 1) + t + r * 64
                term = kpad[o:o + 64, :] * sk[KS - 1 - t:KS - t, :]
                acc = term if acc is None else acc + term
            _st(xin, slice(r * P, r * P + 64), (0, 1), acc * v_ref[r * 64:(r + 1) * 64, cs].astype(F32))

        def s1(i, carry):
            ns = [i * 4 + u for u in range(4)]
            xs = [_ld(xin, pl.ds(n2, 32, stride=P), range(4)).astype(BF16) for n2 in ns]
            zs = [_dot(f1_ref[...], x) for x in xs]
            for n2, z in zip(ns, zs):
                _st(abuf, pl.ds(n2, R, stride=P), range(4), z)
            return carry
        jax.lax.fori_loop(0, 16, s1, 0)

        def s2(i, carry):
            ks = [i * 3 + u for u in range(3)]
            xs = [(g_ref[k1], gi_ref[k1], jnp.concatenate([_ld(abuf, pl.ds((2 * k1 + u) * P, 64), range(4))
                                    for u in range(2)], axis=0).astype(BF16))
                  for k1 in ks]
            zs = [_dot(g, x) for g, _, x in xs]
            out = []
            for z, (_, gi, _) in zip(zs, xs):
                xr, xi = z[:64, :CT], z[64:, :CT]
                hr, hi = z[:64, CT:], z[64:, CT:]
                yy = jnp.concatenate([xr * hr - xi * hi, xr * hi + xi * hr], axis=0)
                out.append(_dot(gi, yy.astype(BF16)))
            for k1, o in zip(ks, out):
                for u in range(2):
                    _st(bbuf, pl.ds((2 * k1 + u) * P, 64), (0, 1), o[u * 64:(u + 1) * 64])
            return carry
        jax.lax.fori_loop(0, 11, s2, 0)

        def s3(i, carry):
            ns = [i * 8 + u for u in range(8)]
            bs = [_ld(bbuf, pl.ds(n2, R, stride=P), (0, 1)).astype(BF16) for n2 in ns]
            zs = [_dot(fi_ref[...], b) for b in bs]
            for n2, z in zip(ns, zs):
                _st(xin, pl.ds(n2, 32, stride=P), (2, 3), z)
            return carry
        jax.lax.fori_loop(0, 8, s3, 0)
        sd = sd_ref[:, cs]
        for r in range(S // 64):
            rows = slice(r * P, r * P + 64)
            y_ref[r * 64:(r + 1) * 64, cs] = (_ld(xin, rows, (2, 3)) + _ld(xin, rows, (0, 1)) * sd).astype(BF16)
        return carry
    jax.lax.fori_loop(0, D // CT, tile, 0)


def _attention(qt_ref, k_ref, vt_ref, ot_ref, sb, pb, kb, qb, ml):
    nq = S // BQ
    nst = H * nq

    def stage(t):
        t = jnp.minimum(t, nst - 1)
        h = t // nq
        j = t % nq
        q = qt_ref[_ds(h // 4, 64), _ds(j, BQ)]
        r = jax.lax.broadcasted_iota(jnp.int32, (64, BQ), 0)
        qb[...] = jnp.where((r >> 4) == h % 4, q, jnp.uint32(0))

        @pl.when(t % (4 * nq) == 0)
        def _():
            kb[...] = k_ref[h // 4]

    def step(t, sn, sc, pc, pp):
        tp = jnp.maximum(t - 1, 0)
        hp = tp // nq
        jp = tp % nq
        vt = vt_ref[_ds(hp, 16), :]
        qm = _upk(qb[...])
        m = ml[0:1]
        m8 = l8 = acc = dep = None
        for c in range(S // CK):
            rows = slice(c * CK, (c + 1) * CK)
            prows = slice(c * CK // 2, (c + 1) * CK // 2)
            kc = kb[prows, :]
            if dep is not None:
                kc = jnp.where(jnp.tile(dep, (CK // 16, 1)), jnp.uint32(0), kc)
            s = _dot(_upk(kc), qm)
            sn[rows, :] = s
            mc = jnp.max(s.reshape(CK // 8, 8, BQ), axis=0)
            m8 = mc if m8 is None else jnp.maximum(m8, mc)
            a = _dot(_upk(vt[:, rows]), _upk(pp[prows, :]))
            acc = a if acc is None else acc + a
            p = jnp.exp2(sc[rows, :] - m)
            pc[prows, :] = _pk(p.astype(BF16))
            lc = jnp.sum(p.reshape(CK // 8, 8, BQ), axis=0)
            l8 = lc if l8 is None else l8 + lc
            dep = functools.reduce(
                jnp.minimum, [lc[:, i * 128:(i + 1) * 128] for i in range(BQ // 128)]) < -1.0
        ot_ref[_ds(hp, 32), _ds(jp, BQ)] = (acc / ml[1:2]).astype(BF16)
        ml[0:1] = jnp.max(m8, axis=0, keepdims=True)
        ml[1:2] = jnp.sum(l8, axis=0, keepdims=True)

    stage(0)
    qm = _upk(qb[...])
    m8 = None
    for c in range(S // 512):
        s = _dot(_upk(kb[c * 256:(c + 1) * 256, :]), qm)
        sb[0][c * 512:(c + 1) * 512, :] = s
        mc = jnp.max(s.reshape(64, 8, BQ), axis=0)
        m8 = mc if m8 is None else jnp.maximum(m8, mc)
    ml[0:1] = jnp.max(m8, axis=0, keepdims=True)
    ml[1:2] = jnp.ones((1, BQ), F32)
    pb[1][...] = jnp.zeros(pb[1].shape, U32)
    stage(1)

    def body(t, carry):
        for par in (0, 1):
            @pl.when(t % 2 == par)
            def _():
                step(t, sb[1 - par], sb[par], pb[par], pb[1 - par])
        stage(t + 2)
        return carry
    jax.lax.fori_loop(0, nst, body, 0)
    a = _dot(_upk(vt_ref[(H - 1) * 16:H * 16, :]), _upk(pb[1][...]))
    ot_ref[(H - 1) * 32:, (nq - 1) * BQ:] = (a / ml[1:2]).astype(BF16)


def _kernel(x_hbm, wqkv_hbm, wo_hbm, k_hbm, v_hbm, sk_ref, h_hbm, sd_ref,
            f1_ref, fi_ref, g_ref, gi_ref, o_ref,
            xr, y, wt, qt, kk, vt, ot, s0, s1, p0, p1, kb, qb, ml, xin, abuf, bbuf, kpad,
            x_ref, wqkv_ref, wo_ref, k_ref, v_ref, h_ref, sems, wsem):
    def tile_copies(c):
        cs = _ds(c, CT)
        return [pltpu.make_async_copy(k_hbm.at[:, cs], k_ref.at[:, cs], sems.at[0, c]),
                pltpu.make_async_copy(v_hbm.at[:, cs], v_ref.at[:, cs], sems.at[1, c]),
                pltpu.make_async_copy(h_hbm.at[cs, :], h_ref.at[cs, :], sems.at[2, c])]

    def wait_tile(c):
        for cp in tile_copies(c):
            cp.wait()

    rest = [pltpu.make_async_copy(a, b, wsem.at[i]) for i, (a, b) in enumerate(
        ((x_hbm, x_ref), (wqkv_hbm, wqkv_ref), (wo_hbm, wo_ref)))]
    for c in range(D // CT):
        for cp in tile_copies(c):
            cp.start()
    for cp in rest:
        cp.start()
    _conv(k_ref, v_ref, sk_ref, h_ref, sd_ref, f1_ref, fi_ref, g_ref, gi_ref, y,
          xin, abuf, bbuf, kpad, wait_tile)
    for cp in rest:
        cp.wait()

    def wtr(i, carry):
        for s, o in ((0, 0), (2 * D, D)):
            w = wqkv_ref[:, pl.ds(pl.multiple_of(s + i * 128, 128), 128)].astype(F32)
            wt[pl.ds(pl.multiple_of(o + i * 128, 128), 128), :] = w.T.astype(BF16)
        return carry
    jax.lax.fori_loop(0, D // 128, wtr, 0)
    xr[...] = x_ref[...].astype(F32)
    qscale = float(DH ** -0.5 * np.log2(np.e))
    nt = (((1,), (1,)), ((), ()))

    def layer(li, carry):
        def proj(r, carry):
            rows = _ds(r, RB)
            h = _ln(xr[rows, :]).astype(BF16)
            qv = jax.lax.dot_general(wt[...], h, nt, preferred_element_type=F32)
            qt[:, rows] = _pk((qv[:D] * qscale).astype(BF16))
            vt[:, rows] = _pk(qv[D:].astype(BF16))
            kx = _pk(_dot(h, wqkv_ref[:, D:2 * D]).astype(BF16))
            for g in range(8):
                kk[g, _ds(r, RB // 2), :] = kx[:, g * 128:(g + 1) * 128]
            return carry
        jax.lax.fori_loop(0, S // RB, proj, 0)
        _attention(qt, kk, vt, ot, (s0, s1), (p0, p1), kb, qb, ml)

        def post(r, carry):
            rows = _ds(r, RB)
            a = jax.lax.dot_general(ot[:, rows], wo_ref[...], (((0,), (0,)), ((), ())),
                                    preferred_element_type=F32)
            x = xr[rows, :] + a
            x = x + _ln(x) * y[rows, :].astype(F32)
            xr[rows, :] = x
            o_ref[rows, :] = x.astype(BF16)
            return carry
        jax.lax.fori_loop(0, S // RB, post, 0)
        return carry
    jax.lax.fori_loop(0, 2, layer, 0)


@jax.jit
def pallas_interleave_layers__softmax_full_mha__ssm_conv_h3__prompt_kernel(
    A_x, A_wqkv, A_wo, B_q, B_k, B_v, B_shift_k, B_ssm_k, B_ssm_D,
):
    V = pltpu.VMEM
    anyspec = pl.BlockSpec(memory_space=pl.ANY)
    vspec = pl.BlockSpec(memory_space=pltpu.VMEM)
    consts = [c.astype(BF16) for c in _dft_consts()]
    out = pl.pallas_call(
        _kernel,
        in_specs=[anyspec] * 5 + [vspec, anyspec] + [vspec] * 5,
        out_shape=jax.ShapeDtypeStruct((S, D), BF16),
        scratch_shapes=[
            V((S, D), F32), V((S, D), BF16), V((2 * D, D), BF16),
            V((D // 2, S), U32), V((8, S // 2, 128), U32), V((D // 2, S), U32), V((D, S), BF16),
            V((S, BQ), F32), V((S, BQ), F32), V((S // 2, BQ), U32), V((S // 2, BQ), U32),
            V((S // 2, 128), U32), V((64, BQ), U32), V((8, BQ), F32),
            V((4, 32 * P, 128), F32), V((4, R * P, 128), F32), V((2, R * P, 128), F32),
            V((S + 8, CT), F32),
            V((S, D), BF16), V((D, 3 * D), BF16), V((D, D), BF16),
            V((S, D), BF16), V((S, D), BF16), V((D, S), BF16),
            pltpu.SemaphoreType.DMA((3, D // CT)), pltpu.SemaphoreType.DMA((3,)),
        ],
        compiler_params=pltpu.CompilerParams(vmem_limit_bytes=120 << 20),
    )(A_x.reshape(S, D), A_wqkv, A_wo, B_k.reshape(S, D), B_v.reshape(S, D),
      B_shift_k.T.astype(F32), B_ssm_k, B_ssm_D.reshape(1, D).astype(F32), *consts)
    return out.reshape(1, S, D)
```

```python
import functools
import numpy as np
import jax
import jax.numpy as jnp
import jax.experimental.pallas as pl
import jax.experimental.pallas.tpu as pltpu

S, D, H, DH, KS = 2048, 1024, 32, 32, 4
BQ, CK, RB, CT = 512, 128, 512, 256
R = 72
P = 65
F32, BF16, U32 = jnp.float32, jnp.bfloat16, jnp.uint32


def _dft_consts():
    n = 4096
    k1 = np.arange(33)[:, None]
    n1 = np.arange(32)[None, :]
    f1 = np.zeros((R, 32))
    f1[0:66:2] = np.cos(2 * np.pi * k1 * n1 / 64)
    f1[1:66:2] = -np.sin(2 * np.pi * k1 * n1 / 64)
    wgt = np.where((k1 == 0) | (k1 == 32), 1.0, 2.0)
    fi = np.zeros((32, R))
    fi[:, 0:66:2] = (wgt * np.cos(2 * np.pi * k1 * n1 / 64)).T / 64
    fi[:, 1:66:2] = (-wgt * np.sin(2 * np.pi * k1 * n1 / 64)).T / 64
    a = np.arange(64)
    g = np.zeros((33, 128, 128))
    gi = np.zeros((33, 128, 128))
    for k in range(33):
        w = np.exp(-2j * np.pi * (a[:, None] * a[None, :] / 64 + k * a[None, :] / n))
        g[k] = np.block([[w.real, -w.imag], [w.imag, w.real]])
        wi = np.conj(w).T / 64
        gi[k] = np.block([[wi.real, -wi.imag], [wi.imag, wi.real]])
    return [x.astype(np.float32) for x in (f1, fi, g, gi)]


def _pk(x):
    return pltpu.bitcast(x, U32)


def _upk(x):
    return pltpu.bitcast(x, BF16)


def _dot(a, b):
    return jnp.dot(a, b, preferred_element_type=F32)


def _ln(x):
    m = jnp.mean(x, axis=-1, keepdims=True)
    d = x - m
    v = jnp.mean(d * d, axis=-1, keepdims=True)
    return d * jax.lax.rsqrt(v + 1e-5)


def _ds(i, n):
    return pl.ds(pl.multiple_of(i * n, n), n)


def _ld(ref, rows, js):
    return jnp.concatenate([ref[j, rows, :] for j in js], axis=1)


def _st(ref, rows, js, val):
    for i, j in enumerate(js):
        ref[j, rows, :] = val[:, i * 128:(i + 1) * 128]


def _conv(k_ref, v_ref, sk_ref, h_ref, sd_ref, f1_ref, fi_ref, g_ref, gi_ref, y_ref,
          xin, abuf, bbuf, kpad, vst, hst, wait_tile):
    bbuf[:, 66 * P:, :] = jnp.zeros((2, (R - 66) * P, 128), F32)
    kpad[0:8, :] = jnp.zeros((8, CT), F32)

    def tile(c, carry):
        cs = _ds(c, CT)
        wait_tile(c)
        kpad[8:, :] = k_ref[:, cs].astype(F32)
        vst[...] = v_ref[:, cs]
        hst[...] = h_ref[cs, :]
        sk = sk_ref[:, cs]

        @pl.when(c >= 0)
        def _():
            for r in range(S // 128):
                ht = hst[:, r * 128:(r + 1) * 128].astype(F32).T
                for u in range(2):
                    b = 2 * r + u
                    rows = slice(b * P, b * P + 64)
                    _st(xin, rows, (2, 3), ht[u * 64:(u + 1) * 64])
                    acc = None
                    for t in range(KS):
                        o = 8 - (KS - 1) + t + b * 64
                        term = kpad[o:o + 64, :] * sk[KS - 1 - t:KS - t, :]
                        acc = term if acc is None else acc + term
                    _st(xin, rows, (0, 1), acc * vst[b * 64:(b + 1) * 64, :].astype(F32))

        def s1(i, carry):
            ns = [i * 8 + u for u in range(8)]
            xs = [_ld(xin, pl.ds(n2, 32, stride=P), range(4)).astype(BF16) for n2 in ns]
            zs = [_dot(f1_ref[...], x) for x in xs]
            for n2, z in zip(ns, zs):
                _st(abuf, pl.ds(n2, R, stride=P), range(4), z)
            return carry
        jax.lax.fori_loop(0, 8, s1, 0)

        def s2(i, carry):
            ks = [i * 3 + u for u in range(3)]
            xs = [(g_ref[k1], gi_ref[k1], jnp.concatenate([_ld(abuf, pl.ds((2 * k1 + u) * P, 64), range(4))
                                    for u in range(2)], axis=0).astype(BF16))
                  for k1 in ks]
            zs = [_dot(g, x) for g, _, x in xs]
            out = []
            for z, (_, gi, _) in zip(zs, xs):
                xr, xi = z[:64, :CT], z[64:, :CT]
                hr, hi = z[:64, CT:], z[64:, CT:]
                yy = jnp.concatenate([xr * hr - xi * hi, xr * hi + xi * hr], axis=0)
                out.append(_dot(gi, yy.astype(BF16)))
            for k1, o in zip(ks, out):
                for u in range(2):
                    _st(bbuf, pl.ds((2 * k1 + u) * P, 64), (0, 1), o[u * 64:(u + 1) * 64])
            return carry
        jax.lax.fori_loop(0, 11, s2, 0)

        def s3(i, carry):
            ns = [i * 16 + u for u in range(16)]
            bs = [_ld(bbuf, pl.ds(n2, R, stride=P), (0, 1)).astype(BF16) for n2 in ns]
            zs = [_dot(fi_ref[...], b) for b in bs]
            for n2, z in zip(ns, zs):
                _st(xin, pl.ds(n2, 32, stride=P), (2, 3), z)
            return carry
        jax.lax.fori_loop(0, 4, s3, 0)
        sd = sd_ref[:, cs]
        for r in range(S // 64):
            rows = slice(r * P, r * P + 64)
            y_ref[r * 64:(r + 1) * 64, cs] = (_ld(xin, rows, (2, 3)) + _ld(xin, rows, (0, 1)) * sd).astype(BF16)
        return carry
    jax.lax.fori_loop(0, D // CT, tile, 0)


def _attention(qt_ref, k_ref, vt_ref, ot_ref, sb, pb, kb, qb, ml):
    nq = S // BQ
    nst = H * nq

    def stage(t):
        t = jnp.minimum(t, nst - 1)
        h = t // nq
        j = t % nq
        q = qt_ref[_ds(h // 4, 64), _ds(j, BQ)]
        r = jax.lax.broadcasted_iota(jnp.int32, (64, BQ), 0)
        qb[...] = jnp.where((r >> 4) == h % 4, q, jnp.uint32(0))

        @pl.when(t % (4 * nq) == 0)
        def _():
            kb[...] = k_ref[h // 4]

    def step(t, sn, sc, pc, pp):
        tp = jnp.maximum(t - 1, 0)
        hp = tp // nq
        jp = tp % nq
        vt = vt_ref[_ds(hp, 16), :]
        qm = _upk(qb[...])
        m = ml[0:1]
        m8 = l8 = acc = dep = None
        for c in range(S // CK):
            rows = slice(c * CK, (c + 1) * CK)
            prows = slice(c * CK // 2, (c + 1) * CK // 2)
            kc = kb[prows, :]
            if dep is not None:
                kc = jnp.where(jnp.tile(dep, (CK // 16, 1)), jnp.uint32(0), kc)
            s = _dot(_upk(kc), qm)
            sn[rows, :] = s
            mc = jnp.max(s.reshape(CK // 8, 8, BQ), axis=0)
            m8 = mc if m8 is None else jnp.maximum(m8, mc)
            a = _dot(_upk(vt[:, rows]), _upk(pp[prows, :]))
            acc = a if acc is None else acc + a
            p = jnp.exp2(sc[rows, :] - m)
            pc[prows, :] = _pk(p.astype(BF16))
            lc = jnp.sum(p.reshape(CK // 8, 8, BQ), axis=0)
            l8 = lc if l8 is None else l8 + lc
            dep = functools.reduce(
                jnp.minimum, [lc[:, i * 128:(i + 1) * 128] for i in range(BQ // 128)]) < -1.0
        ot_ref[_ds(hp, 32), _ds(jp, BQ)] = (acc / ml[1:2]).astype(BF16)
        ml[0:1] = jnp.max(m8, axis=0, keepdims=True)
        ml[1:2] = jnp.sum(l8, axis=0, keepdims=True)

    stage(0)
    qm = _upk(qb[...])
    m8 = None
    for c in range(S // 512):
        s = _dot(_upk(kb[c * 256:(c + 1) * 256, :]), qm)
        sb[0][c * 512:(c + 1) * 512, :] = s
        mc = jnp.max(s.reshape(64, 8, BQ), axis=0)
        m8 = mc if m8 is None else jnp.maximum(m8, mc)
    ml[0:1] = jnp.max(m8, axis=0, keepdims=True)
    ml[1:2] = jnp.ones((1, BQ), F32)
    pb[1][...] = jnp.zeros(pb[1].shape, U32)
    stage(1)

    def body(t, carry):
        for par in (0, 1):
            @pl.when(t % 2 == par)
            def _():
                step(t, sb[1 - par], sb[par], pb[par], pb[1 - par])
        stage(t + 2)
        return carry
    jax.lax.fori_loop(0, nst, body, 0)
    a = _dot(_upk(vt_ref[(H - 1) * 16:H * 16, :]), _upk(pb[1][...]))
    ot_ref[(H - 1) * 32:, (nq - 1) * BQ:] = (a / ml[1:2]).astype(BF16)


def _kernel(x_hbm, wqkv_hbm, wo_hbm, k_hbm, v_hbm, sk_ref, h_hbm, sd_ref,
            f1_ref, fi_ref, g_ref, gi_ref, o_ref,
            xr, y, wt, qt, kk, vt, ot, s0, s1, p0, p1, kb, qb, ml, xin, abuf, bbuf, kpad,
            x_ref, wqkv_ref, wo_ref, k_ref, v_ref, h_ref, sems, wsem, vst, hst, ob, osem):
    def tile_copies(c):
        cs = _ds(c, CT)
        return [pltpu.make_async_copy(k_hbm.at[:, cs], k_ref.at[:, cs], sems.at[0, c]),
                pltpu.make_async_copy(v_hbm.at[:, cs], v_ref.at[:, cs], sems.at[1, c]),
                pltpu.make_async_copy(h_hbm.at[cs, :], h_ref.at[cs, :], sems.at[2, c])]

    def wait_tile(c):
        for cp in tile_copies(c):
            cp.wait()

    rest = [pltpu.make_async_copy(a, b, wsem.at[i]) for i, (a, b) in enumerate(
        ((x_hbm, x_ref), (wqkv_hbm, wqkv_ref), (wo_hbm, wo_ref)))]
    for c in range(D // CT):
        for cp in tile_copies(c):
            cp.start()
    for cp in rest:
        cp.start()
    _conv(k_ref, v_ref, sk_ref, h_ref, sd_ref, f1_ref, fi_ref, g_ref, gi_ref, y,
          xin, abuf, bbuf, kpad, vst, hst, wait_tile)
    for cp in rest:
        cp.wait()

    def wtr(i, carry):
        for s, o in ((0, 0), (2 * D, D)):
            w = wqkv_ref[:, pl.ds(pl.multiple_of(s + i * 128, 128), 128)].astype(F32)
            wt[pl.ds(pl.multiple_of(o + i * 128, 128), 128), :] = w.T.astype(BF16)
        return carry
    jax.lax.fori_loop(0, D // 128, wtr, 0)
    xr[...] = x_ref[...].astype(F32)
    qscale = float(DH ** -0.5 * np.log2(np.e))
    nt = (((1,), (1,)), ((), ()))

    def out_copy(r):
        return pltpu.make_async_copy(ob.at[_ds(r, RB)], o_ref.at[_ds(r, RB)], osem.at[r])

    def layer(li, carry):
        def proj(r, carry):
            rows = _ds(r, RB)
            h = _ln(xr[rows, :]).astype(BF16)
            qv = jax.lax.dot_general(wt[...], h, nt, preferred_element_type=F32)
            qt[:, rows] = _pk((qv[:D] * qscale).astype(BF16))
            vt[:, rows] = _pk(qv[D:].astype(BF16))
            kx = _pk(_dot(h, wqkv_ref[:, D:2 * D]).astype(BF16))
            for g in range(8):
                kk[g, _ds(r, RB // 2), :] = kx[:, g * 128:(g + 1) * 128]
            return carry
        jax.lax.fori_loop(0, S // RB, proj, 0)
        _attention(qt, kk, vt, ot, (s0, s1), (p0, p1), kb, qb, ml)

        def post(r, carry):
            rows = _ds(r, RB)
            a = jax.lax.dot_general(ot[:, rows], wo_ref[...], (((0,), (0,)), ((), ())),
                                    preferred_element_type=F32)
            x = xr[rows, :] + a
            x = x + _ln(x) * y[rows, :].astype(F32)
            xr[rows, :] = x

            @pl.when(li == 1)
            def _():
                ob[rows, :] = xr[rows, :].astype(BF16)
                out_copy(r).start()
            return carry
        jax.lax.fori_loop(0, S // RB, post, 0)
        return carry
    jax.lax.fori_loop(0, 2, layer, 0)
    for r in range(S // RB):
        out_copy(r).wait()


@jax.jit
def pallas_interleave_layers__softmax_full_mha__ssm_conv_h3__prompt_kernel(
    A_x, A_wqkv, A_wo, B_q, B_k, B_v, B_shift_k, B_ssm_k, B_ssm_D,
):
    V = pltpu.VMEM
    anyspec = pl.BlockSpec(memory_space=pl.ANY)
    vspec = pl.BlockSpec(memory_space=pltpu.VMEM)
    consts = [c.astype(BF16) for c in _dft_consts()]
    out = pl.pallas_call(
        _kernel,
        in_specs=[anyspec] * 5 + [vspec, anyspec] + [vspec] * 5,
        out_specs=anyspec,
        out_shape=jax.ShapeDtypeStruct((S, D), BF16),
        scratch_shapes=[
            V((S, D), F32), V((S, D), BF16), V((2 * D, D), BF16),
            V((D // 2, S), U32), V((8, S // 2, 128), U32), V((D // 2, S), U32), V((D, S), BF16),
            V((S, BQ), F32), V((S, BQ), F32), V((S // 2, BQ), U32), V((S // 2, BQ), U32),
            V((S // 2, 128), U32), V((64, BQ), U32), V((8, BQ), F32),
            V((4, 32 * P, 128), F32), V((4, R * P, 128), F32), V((2, R * P, 128), F32),
            V((S + 8, CT), F32),
            V((S, D), BF16), V((D, 3 * D), BF16), V((D, D), BF16),
            V((S, D), BF16), V((S, D), BF16), V((D, S), BF16),
            pltpu.SemaphoreType.DMA((3, D // CT)), pltpu.SemaphoreType.DMA((3,)),
            V((S, CT), BF16), V((CT, S), BF16), V((S, D), BF16), pltpu.SemaphoreType.DMA((S // RB,)),
        ],
        compiler_params=pltpu.CompilerParams(vmem_limit_bytes=120 << 20),
    )(A_x.reshape(S, D), A_wqkv, A_wo, B_k.reshape(S, D), B_v.reshape(S, D),
      B_shift_k.T.astype(F32), B_ssm_k, B_ssm_D.reshape(1, D).astype(F32), *consts)
    return out.reshape(1, S, D)
```

```python
import functools
import numpy as np
import jax
import jax.numpy as jnp
import jax.experimental.pallas as pl
import jax.experimental.pallas.tpu as pltpu

S, D, H, DH, KS = 2048, 1024, 32, 32, 4
BQ, CK, RB, CT = 512, 128, 512, 256
R = 72
P = 65
F32, BF16, U32 = jnp.float32, jnp.bfloat16, jnp.uint32


def _dft_consts():
    n = 4096
    k1 = np.arange(33)[:, None]
    n1 = np.arange(32)[None, :]
    f1 = np.zeros((R, 32))
    f1[0:66:2] = np.cos(2 * np.pi * k1 * n1 / 64)
    f1[1:66:2] = -np.sin(2 * np.pi * k1 * n1 / 64)
    wgt = np.where((k1 == 0) | (k1 == 32), 1.0, 2.0)
    fi = np.zeros((32, R))
    fi[:, 0:66:2] = (wgt * np.cos(2 * np.pi * k1 * n1 / 64)).T / 64
    fi[:, 1:66:2] = (-wgt * np.sin(2 * np.pi * k1 * n1 / 64)).T / 64
    a = np.arange(64)
    g = np.zeros((33, 128, 128))
    gi = np.zeros((33, 128, 128))
    for k in range(33):
        w = np.exp(-2j * np.pi * (a[:, None] * a[None, :] / 64 + k * a[None, :] / n))
        g[k] = np.block([[w.real, -w.imag], [w.imag, w.real]])
        wi = np.conj(w).T / 64
        gi[k] = np.block([[wi.real, -wi.imag], [wi.imag, wi.real]])
    return [x.astype(np.float32) for x in (f1, fi, g, gi)]


def _pk(x):
    return pltpu.bitcast(x, U32)


def _upk(x):
    return pltpu.bitcast(x, BF16)


def _dot(a, b):
    return jnp.dot(a, b, preferred_element_type=F32)


def _ln(x):
    m = jnp.mean(x, axis=-1, keepdims=True)
    d = x - m
    v = jnp.mean(d * d, axis=-1, keepdims=True)
    return d * jax.lax.rsqrt(v + 1e-5)


def _ds(i, n):
    return pl.ds(pl.multiple_of(i * n, n), n)


def _ld(ref, rows, js):
    return jnp.concatenate([ref[j, rows, :] for j in js], axis=1)


def _st(ref, rows, js, val):
    for i, j in enumerate(js):
        ref[j, rows, :] = val[:, i * 128:(i + 1) * 128]


def _conv(k_ref, v_ref, sk_ref, h_ref, sd_ref, f1_ref, fi_ref, g_ref, gi_ref, y_ref,
          xin, abuf, bbuf, kpad, vst, hst, wait_tile):
    bbuf[:, 66 * P:, :] = jnp.zeros((2, (R - 66) * P, 128), F32)
    kpad[0:8, :] = jnp.zeros((8, CT), F32)

    def tile(c, carry):
        cs = _ds(c, CT)
        wait_tile(c)
        kpad[8:, :] = k_ref[:, cs].astype(F32)
        vst[...] = v_ref[:, cs]
        hst[...] = h_ref[cs, :]
        sk = sk_ref[:, cs]

        @pl.when(c >= 0)
        def _():
            for r in range(S // 128):
                ht = hst[:, r * 128:(r + 1) * 128].astype(F32).T
                for u in range(2):
                    b = 2 * r + u
                    rows = slice(b * P, b * P + 64)
                    _st(xin, rows, (2, 3), ht[u * 64:(u + 1) * 64])
                    acc = None
                    for t in range(KS):
                        o = 8 - (KS - 1) + t + b * 64
                        term = kpad[o:o + 64, :] * sk[KS - 1 - t:KS - t, :]
                        acc = term if acc is None else acc + term
                    _st(xin, rows, (0, 1), acc * vst[b * 64:(b + 1) * 64, :].astype(F32))

        def s1(i, carry):
            ns = [i * 8 + u for u in range(8)]
            xs = [_ld(xin, pl.ds(n2, 32, stride=P), range(4)).astype(BF16) for n2 in ns]
            zs = [_dot(f1_ref[...], x) for x in xs]
            for n2, z in zip(ns, zs):
                _st(abuf, pl.ds(n2, R, stride=P), range(4), z)
            return carry
        jax.lax.fori_loop(0, 8, s1, 0)

        def s2(i, carry):
            ks = [i * 3 + u for u in range(3)]
            xs = [(g_ref[k1], gi_ref[k1], jnp.concatenate([_ld(abuf, pl.ds((2 * k1 + u) * P, 64), range(4))
                                    for u in range(2)], axis=0).astype(BF16))
                  for k1 in ks]
            zs = [_dot(g, x) for g, _, x in xs]
            out = []
            for z, (_, gi, _) in zip(zs, xs):
                xr, xi = z[:64, :CT], z[64:, :CT]
                hr, hi = z[:64, CT:], z[64:, CT:]
                yy = jnp.concatenate([xr * hr - xi * hi, xr * hi + xi * hr], axis=0)
                out.append(_dot(gi, yy.astype(BF16)))
            for k1, o in zip(ks, out):
                for u in range(2):
                    _st(bbuf, pl.ds((2 * k1 + u) * P, 64), (0, 1), o[u * 64:(u + 1) * 64])
            return carry
        jax.lax.fori_loop(0, 11, s2, 0)

        def s3(i, carry):
            ns = [i * 16 + u for u in range(16)]
            bs = [_ld(bbuf, pl.ds(n2, R, stride=P), (0, 1)).astype(BF16) for n2 in ns]
            zs = [_dot(fi_ref[...], b) for b in bs]
            for n2, z in zip(ns, zs):
                _st(xin, pl.ds(n2, 32, stride=P), (2, 3), z)
            return carry
        jax.lax.fori_loop(0, 4, s3, 0)
        sd = sd_ref[:, cs]
        for r in range(S // 64):
            rows = slice(r * P, r * P + 64)
            y_ref[r * 64:(r + 1) * 64, cs] = (_ld(xin, rows, (2, 3)) + _ld(xin, rows, (0, 1)) * sd).astype(BF16)
        return carry
    jax.lax.fori_loop(0, D // CT, tile, 0)


def _attention(qt_ref, k_ref, vt_ref, ot_ref, sb, pb, kb, qb, ml):
    nq = S // BQ
    nst = H * nq

    def stage(t):
        t = jnp.minimum(t, nst - 1)
        h = t // nq
        j = t % nq
        q = qt_ref[_ds(h // 4, 64), _ds(j, BQ)]
        r = jax.lax.broadcasted_iota(jnp.int32, (64, BQ), 0)
        qb[...] = jnp.where((r >> 4) == h % 4, q, jnp.uint32(0))

        @pl.when(t % (4 * nq) == 0)
        def _():
            kb[...] = k_ref[h // 4]

    def step(t, sn, sc, pc, pp):
        tp = jnp.maximum(t - 1, 0)
        hp = tp // nq
        jp = tp % nq
        vt = vt_ref[_ds(hp, 16), :]
        qm = _upk(qb[...])
        m = ml[0:1]
        m8 = l8 = acc = dep = None
        for c in range(S // CK):
            rows = slice(c * CK, (c + 1) * CK)
            prows = slice(c * CK // 2, (c + 1) * CK // 2)
            kc = kb[prows, :]
            if dep is not None:
                kc = jnp.where(jnp.tile(dep, (CK // 16, 1)), jnp.uint32(0), kc)
            s = _dot(_upk(kc), qm)
            sn[rows, :] = s
            mc = jnp.max(s.reshape(CK // 8, 8, BQ), axis=0)
            m8 = mc if m8 is None else jnp.maximum(m8, mc)
            a = _dot(_upk(vt[:, rows]), _upk(pp[prows, :]))
            acc = a if acc is None else acc + a
            p = jnp.exp2(sc[rows, :] - m)
            pc[prows, :] = _pk(p.astype(BF16))
            lc = jnp.sum(p.reshape(CK // 8, 8, BQ), axis=0)
            l8 = lc if l8 is None else l8 + lc
            dep = functools.reduce(
                jnp.minimum, [lc[:, i * 128:(i + 1) * 128] for i in range(BQ // 128)]) < -1.0
        ot_ref[_ds(hp, 32), _ds(jp, BQ)] = (acc / ml[1:2]).astype(BF16)
        ml[0:1] = jnp.max(m8, axis=0, keepdims=True)
        ml[1:2] = jnp.sum(l8, axis=0, keepdims=True)

    stage(0)
    qm = _upk(qb[...])
    m8 = None
    for c in range(S // 512):
        s = _dot(_upk(kb[c * 256:(c + 1) * 256, :]), qm)
        sb[0][c * 512:(c + 1) * 512, :] = s
        mc = jnp.max(s.reshape(64, 8, BQ), axis=0)
        m8 = mc if m8 is None else jnp.maximum(m8, mc)
    ml[0:1] = jnp.max(m8, axis=0, keepdims=True)
    ml[1:2] = jnp.ones((1, BQ), F32)
    pb[1][...] = jnp.zeros(pb[1].shape, U32)
    stage(1)

    def body(t, carry):
        for par in (0, 1):
            @pl.when(t % 2 == par)
            def _():
                step(t, sb[1 - par], sb[par], pb[par], pb[1 - par])
        stage(t + 2)
        return carry
    jax.lax.fori_loop(0, nst, body, 0)
    a = _dot(_upk(vt_ref[(H - 1) * 16:H * 16, :]), _upk(pb[1][...]))
    ot_ref[(H - 1) * 32:, (nq - 1) * BQ:] = (a / ml[1:2]).astype(BF16)


def _kernel(x_hbm, wqkv_hbm, wo_hbm, k_hbm, v_hbm, sk_ref, h_hbm, sd_ref,
            f1_ref, fi_ref, g_ref, gi_ref, o_ref,
            xr, y, wt, qt, kk, vt, ot, s0, s1, p0, p1, kb, qb, ml, xin, abuf, bbuf, kpad,
            x_ref, wqkv_ref, wo_ref, k_ref, v_ref, h_ref, sems, wsem, vst, hst, ob, osem):
    def tile_copies(c):
        cs = _ds(c, CT)
        return [pltpu.make_async_copy(k_hbm.at[:, cs], k_ref.at[:, cs], sems.at[0, c]),
                pltpu.make_async_copy(v_hbm.at[:, cs], v_ref.at[:, cs], sems.at[1, c]),
                pltpu.make_async_copy(h_hbm.at[cs, :], h_ref.at[cs, :], sems.at[2, c])]

    def wait_tile(c):
        for cp in tile_copies(c):
            cp.wait()

    rest = [pltpu.make_async_copy(a, b, wsem.at[i]) for i, (a, b) in enumerate(
        ((x_hbm, x_ref), (wqkv_hbm, wqkv_ref), (wo_hbm, wo_ref)))]
    for c in range(D // CT):
        for cp in tile_copies(c):
            cp.start()
    for cp in rest:
        cp.start()
    _conv(k_ref, v_ref, sk_ref, h_ref, sd_ref, f1_ref, fi_ref, g_ref, gi_ref, y,
          xin, abuf, bbuf, kpad, vst, hst, wait_tile)
    for cp in rest:
        cp.wait()

    def wtr(i, carry):
        for s, o in ((0, 0), (2 * D, D)):
            w = wqkv_ref[:, pl.ds(pl.multiple_of(s + i * 128, 128), 128)].astype(F32)
            wt[pl.ds(pl.multiple_of(o + i * 128, 128), 128), :] = w.T.astype(BF16)
        return carry
    jax.lax.fori_loop(0, D // 128, wtr, 0)
    xr[...] = x_ref[...].astype(F32)
    qscale = float(DH ** -0.5 * np.log2(np.e))
    nt = (((1,), (1,)), ((), ()))

    def out_copy(r):
        return pltpu.make_async_copy(ob.at[_ds(r, RB)], o_ref.at[_ds(r, RB)], osem.at[r])

    def layer(li, carry):
        def proj(r, carry):
            rows = _ds(r, RB)
            h = _ln(xr[rows, :]).astype(BF16)
            qv = jax.lax.dot_general(wt[...], h, nt, preferred_element_type=F32)
            qt[:, rows] = _pk((qv[:D] * qscale).astype(BF16))
            vt[:, rows] = _pk(qv[D:].astype(BF16))
            kx = _pk(_dot(h, wqkv_ref[:, D:2 * D]).astype(BF16))
            for g in range(8):
                kk[g, _ds(r, RB // 2), :] = kx[:, g * 128:(g + 1) * 128]
            return carry
        jax.lax.fori_loop(0, S // RB, proj, 0)
        _attention(qt, kk, vt, ot, (s0, s1), (p0, p1), kb, qb, ml)

        def post(r, carry):
            rows = _ds(r, RB)
            n = RB // 128
            subs = [_ds(r * n + u, 128) for u in range(n)]
            ins = [(ot[:, t], xr[t, :], y[t, :]) for t in subs]
            outs = []
            for o, x, yy in ins:
                x = x + jax.lax.dot_general(o, wo_ref[...], (((0,), (0,)), ((), ())),
                                            preferred_element_type=F32)
                outs.append(x + _ln(x) * yy.astype(F32))
            for t, x in zip(subs, outs):
                xr[t, :] = x

            @pl.when(li == 1)
            def _():
                ob[rows, :] = xr[rows, :].astype(BF16)
                out_copy(r).start()
            return carry
        jax.lax.fori_loop(0, S // RB, post, 0)
        return carry
    jax.lax.fori_loop(0, 2, layer, 0)
    for r in range(S // RB):
        out_copy(r).wait()


@jax.jit
def pallas_interleave_layers__softmax_full_mha__ssm_conv_h3__prompt_kernel(
    A_x, A_wqkv, A_wo, B_q, B_k, B_v, B_shift_k, B_ssm_k, B_ssm_D,
):
    V = pltpu.VMEM
    anyspec = pl.BlockSpec(memory_space=pl.ANY)
    vspec = pl.BlockSpec(memory_space=pltpu.VMEM)
    consts = [c.astype(BF16) for c in _dft_consts()]
    out = pl.pallas_call(
        _kernel,
        in_specs=[anyspec] * 5 + [vspec, anyspec] + [vspec] * 5,
        out_specs=anyspec,
        out_shape=jax.ShapeDtypeStruct((S, D), BF16),
        scratch_shapes=[
            V((S, D), F32), V((S, D), BF16), V((2 * D, D), BF16),
            V((D // 2, S), U32), V((8, S // 2, 128), U32), V((D // 2, S), U32), V((D, S), BF16),
            V((S, BQ), F32), V((S, BQ), F32), V((S // 2, BQ), U32), V((S // 2, BQ), U32),
            V((S // 2, 128), U32), V((64, BQ), U32), V((8, BQ), F32),
            V((4, 32 * P, 128), F32), V((4, R * P, 128), F32), V((2, R * P, 128), F32),
            V((S + 8, CT), F32),
            V((S, D), BF16), V((D, 3 * D), BF16), V((D, D), BF16),
            V((S, D), BF16), V((S, D), BF16), V((D, S), BF16),
            pltpu.SemaphoreType.DMA((3, D // CT)), pltpu.SemaphoreType.DMA((3,)),
            V((S, CT), BF16), V((CT, S), BF16), V((S, D), BF16), pltpu.SemaphoreType.DMA((S // RB,)),
        ],
        compiler_params=pltpu.CompilerParams(vmem_limit_bytes=120 << 20),
    )(A_x.reshape(S, D), A_wqkv, A_wo, B_k.reshape(S, D), B_v.reshape(S, D),
      B_shift_k.T.astype(F32), B_ssm_k, B_ssm_D.reshape(1, D).astype(F32), *consts)
    return out.reshape(1, S, D)
```
